```python
import os as _os
_os.environ.setdefault("JAX_PLATFORMS", "cpu")
import jax
import jax.numpy as jnp

def _softmax(x, axis=-1):
    return jax.nn.softmax(x, axis=axis)
def _gelu(x):
    return jax.nn.gelu(x, approximate=True)
def _silu(x):
    return jax.nn.silu(x)
def _sigmoid(x):
    return jax.nn.sigmoid(x)
def _layernorm(x, axis=-1, eps=1e-5):
    m = jnp.mean(x, axis=axis, keepdims=True)
    v = jnp.var(x, axis=axis, keepdims=True)
    return (x - m) / jnp.sqrt(v + eps)
def _scatter_add(tgt, idx, src, axis=0):
    return tgt.at[idx].add(src)
def _segment_sum(src, seg, n):
    return jax.ops.segment_sum(src, seg, n)
class _Rng:
    def __init__(self, key):
        self._k = key
    def _next(self):
        self._k, sub = jax.random.split(self._k)
        return sub
    def normal(self, shape):
        return jax.random.normal(self._next(), shape, dtype=jnp.bfloat16)
    def randint(self, lo, hi, shape):
        return jax.random.randint(self._next(), shape, lo, hi, dtype=jnp.int32)
    def uniform(self, shape, lo=0.0, hi=1.0):
        return jax.random.uniform(self._next(), shape, jnp.bfloat16, lo, hi)
    def permutation(self, n):
        return jax.random.permutation(self._next(), n)


kernel_name = 'sequential_preLN__spectral_gfnet__glu_gated_bilinear__prompt'

def setup_inputs():
    _rng = _Rng(jax.random.key(int.from_bytes(__import__("os").urandom(4), "little")))
    _w = (lambda a: (lambda t: t.astype(jnp.bfloat16) if jnp.issubdtype(t.dtype, jnp.floating) else t)(jnp.asarray(a)))
    def _A_setup():
        B, S, D = 1, 2048, 448
        Df = D // 2 + 1
        return {
            "x": _w((lambda *s: _rng.normal(s) * 0.05)(B, S, D)),
            "w_r": _w((lambda *s: _rng.normal(s) * 0.2)(S, Df) * 0.02),
            "w_i": _w((lambda *s: _rng.normal(s) * 0.2)(S, Df) * 0.02),
        }
    _A_in = _A_setup()

    def _B_setup():
        B, S, D, F = 1, 2048, 448, 1792
        return {
            "x": _w((lambda *s: _rng.normal(s) * 0.05)(B, S, D)),
            "w_gate": _w((lambda *s: _rng.normal(s) * 0.05)(D, F) * (D ** -0.5)),
            "w_up": _w((lambda *s: _rng.normal(s) * 0.05)(D, F) * (D ** -0.5)),
            "w_down": _w((lambda *s: _rng.normal(s) * 0.05)(F, D) * (F ** -0.5)),
        }
    _B_in = _B_setup()

    return {
        "A_x": _A_in["x"],
        "A_w_r": _A_in["w_r"],
        "A_w_i": _A_in["w_i"],
        "B_x": _B_in["x"],
        "B_w_gate": _B_in["w_gate"],
        "B_w_up": _B_in["w_up"],
        "B_w_down": _B_in["w_down"],
    }

def reference(A_x, A_w_r, A_w_i, B_x, B_w_gate, B_w_up, B_w_down):
    def _A_ref(x, w_r, w_i):
        B, S, D = x.shape
        X = (lambda x, axes=(-2,-1): jnp.fft.rfft2(x.astype(jnp.float32), axes=axes))(x, axes=(-2, -1))
        W = w_r + 1j * w_i
        X = X * W
        y = (lambda x, s, axes=(-2,-1): jnp.fft.irfft2(x, s=s, axes=axes).astype(jnp.bfloat16))(X, (S, D), axes=(-2, -1))
        return y

    def _B_ref(x, w_gate, w_up, w_down):
        g = jnp.einsum("bsd,df->bsf", x, w_gate)
        u = jnp.einsum("bsd,df->bsf", x, w_up)
        h = g * u
        return jnp.einsum("bsf,fd->bsd", h, w_down)

    x = A_x
    h = x + _A_ref(_layernorm(x, axis=-1), A_w_r, A_w_i)
    h2 = h + _B_ref(_layernorm(h, axis=-1), B_w_gate, B_w_up, B_w_down)
    return h2
```

```python
import functools

import numpy as np
import jax
import jax.numpy as jnp
import jax.experimental.pallas as pl
import jax.experimental.pallas.tpu as pltpu

S = 2048
D = 448
DF = D // 2 + 1
F = 1792
N1 = 16
N2 = 128
CP = 256
RB = 32
TS = 256
EPS = 1e-5

_C1 = float(np.cos(np.pi / 8))
_C3 = float(np.cos(3 * np.pi / 8))
_R = float(np.sqrt(0.5))


def _ang(a, b, n):
    return 2.0 * np.pi * ((np.outer(a, b)) % n).astype(np.float64) / n


@functools.lru_cache(maxsize=None)
def _constants():
    d = np.arange(D)
    c = np.arange(DF)
    fdt = np.zeros((2 * CP, D))
    fdt[:DF] = np.cos(_ang(c, d, D))
    fdt[CP:CP + DF] = -np.sin(_ang(c, d, D))
    coef = np.full(DF, 2.0)
    coef[0] = 1.0
    coef[-1] = 1.0
    cp = np.zeros((D, CP))
    sp = np.zeros((D, CP))
    cp[:, :DF] = coef[None, :] * np.cos(_ang(d, c, D)) / (S * D)
    sp[:, :DF] = coef[None, :] * np.sin(_ang(d, c, D)) / (S * D)
    ci1t = np.concatenate([cp, -sp], axis=1)
    ci2t = np.concatenate([sp, cp], axis=1)
    n2 = np.arange(N2)
    k2 = np.arange(N2)
    g = np.zeros((N1, N2, 2 * N2))
    gt = np.zeros((N1, N2, 2 * N2))
    for k1 in range(N1):
        a = _ang(k1 + N1 * k2, n2, S)
        g[k1, :, :N2] = np.cos(a)
        g[k1, :, N2:] = -np.sin(a)
        gt[k1, :, :N2] = np.cos(a).T
        gt[k1, :, N2:] = -np.sin(a).T
    pm = np.zeros((N2, N2))
    kk = np.arange(N2)
    pm[kk, (kk % N1) * 8 + kk // N1] = 1.0
    return tuple(np.asarray(v, dtype=np.float32).astype(jnp.bfloat16)
                 for v in (fdt, ci1t, ci2t, gt, g, pm))


def _dot(a, b):
    return jnp.dot(a, b, preferred_element_type=jnp.float32)


def _rdft16(x):
    a = [x[n] + x[n + 8] for n in range(8)]
    b = [x[n] - x[n + 8] for n in range(8)]
    c = [a[n] + a[n + 4] for n in range(4)]
    d = [a[n] - a[n + 4] for n in range(4)]
    e0 = c[0] + c[2]
    e1 = c[1] + c[3]
    x0 = e0 + e1
    x8 = e0 - e1
    x4r = c[0] - c[2]
    x4i = c[3] - c[1]
    p = _R * (d[1] - d[3])
    q = _R * (d[1] + d[3])
    x2r = d[0] + p
    x2i = -(d[2] + q)
    x6r = d[0] - p
    x6i = d[2] - q
    u1, u2, u3 = b[1] - b[7], b[2] - b[6], b[3] - b[5]
    v1, v2, v3 = b[1] + b[7], b[2] + b[6], b[3] + b[5]
    aa = _C1 * u1 + _C3 * u3
    bb = _C3 * u1 - _C1 * u3
    rr = _R * u2
    bp = b[0] + rr
    bm = b[0] - rr
    cc = _C3 * v1 + _C1 * v3
    dd = _C1 * v1 - _C3 * v3
    r2 = _R * v2
    s1 = r2 + b[4]
    s2 = r2 - b[4]
    return [x0, x8,
            bp + aa, -(cc + s1),
            x2r, x2i,
            bm + bb, -(dd + s2),
            x4r, x4i,
            bm - bb, s2 - dd,
            x6r, x6i,
            bp - aa, s1 - cc]


def _irdft16(p, m):
    e0 = p[0] + p[8]
    e1 = p[0] - p[8]
    c = [e0 + p[4], e1 - m[4], e0 - p[4], e1 + m[4]]
    pp = _R * (p[2] - p[6])
    qq = _R * (m[2] + m[6])
    s26 = p[2] + p[6]
    t26 = m[6] - m[2]
    d = [s26, pp - qq, t26, -(pp + qq)]
    ev = [c[0] + d[0], c[1] + d[1], c[2] + d[2], c[3] + d[3],
          c[0] - d[0], c[1] - d[1], c[2] - d[2], c[3] - d[3]]
    a17 = p[1] - p[7]
    a35 = p[3] - p[5]
    k1 = _C1 * a17 + _C3 * a35
    k3 = _C3 * a17 - _C1 * a35
    k2 = _R * ((p[1] + p[7]) - (p[3] + p[5]))
    b17 = m[1] + m[7]
    b35 = m[3] + m[5]
    l1 = _C3 * b17 + _C1 * b35
    l3 = _C1 * b17 - _C3 * b35
    l2 = _R * ((m[1] - m[7]) + (m[3] - m[5]))
    od = [(p[1] + p[7]) + (p[3] + p[5]),
          k1 - l1, k2 - l2, k3 - l3,
          (m[3] - m[1]) + (m[7] - m[5]),
          -(k3 + l3), -(k2 + l2), -(k1 + l1)]
    return [ev[n] + od[n] for n in range(8)] + [ev[n] - od[n] for n in range(8)]


def _kernel(x_ref, wr_hbm, wi_hbm, wg_hbm, wu_hbm, wd_hbm,
            fdt_hbm, ci1_hbm, ci2_hbm, gt_hbm, g_hbm, pm_ref,
            o_ref, a_scr, p_scr, z_scr, b_scr, h_scr, ln2_scr,
            wr_ref, wi_ref, wg_ref, wu_ref, wd_ref,
            fdt_ref, ci1_ref, ci2_ref, gt_ref, g_ref, w_scr, sems):
    bf = jnp.bfloat16
    f32 = jnp.float32

    pairs = [(fdt_hbm, fdt_ref), (gt_hbm, gt_ref), (wr_hbm, wr_ref), (wi_hbm, wi_ref),
             (g_hbm, g_ref), (ci1_hbm, ci1_ref), (ci2_hbm, ci2_ref),
             (wg_hbm, wg_ref), (wu_hbm, wu_ref), (wd_hbm, wd_ref)]
    copies = [pltpu.make_async_copy(src, dst, sems.at[i]) for i, (src, dst) in enumerate(pairs)]
    for cp in copies:
        cp.start()

    xf = x_ref[...].astype(f32)
    mu = jnp.mean(xf, axis=0, keepdims=True)
    xc = xf - mu
    rs = jax.lax.rsqrt(jnp.mean(xc * xc, axis=0, keepdims=True) + EPS)

    for rc in range(D // RB):
        rows = pl.ds(rc * RB, RB)
        blk = [((x_ref[rows, pl.ds(n * N2, N2)].astype(f32) - mu[:, n * N2:(n + 1) * N2])
                * rs[:, n * N2:(n + 1) * N2]).astype(bf).astype(f32) for n in range(N1)]
        outs = _rdft16(blk)
        for sl in range(N1):
            a_scr[rows, pl.ds(sl * N2, N2)] = outs[sl].astype(bf)

    copies[0].wait()
    p_scr[...] = _dot(fdt_ref[...], a_scr[...])
    for cp in copies[1:7]:
        cp.wait()

    zrow = jnp.zeros((CP - DF, N2), f32)
    grp = jax.lax.broadcasted_iota(jnp.int32, (CP, N2), 1) // 8
    for a, src in enumerate((wr_ref, wi_ref)):
        blk = [jnp.concatenate([_dot(src[:, pl.ds(b * N2, N2)], pm_ref[...]), zrow], axis=0)
               for b in range(N1)]
        for t in (8, 4, 2, 1):
            low = (grp & t) == 0
            for b in range(N1):
                if b & t:
                    continue
                lo, hi = blk[b], blk[b + t]
                blk[b] = jnp.where(low, lo, pltpu.roll(hi, 8 * t, 1))
                blk[b + t] = jnp.where(low, pltpu.roll(lo, N2 - 8 * t, 1), hi)
        for b in range(N1):
            w_scr[a, :, pl.ds(b * N2, N2)] = blk[b]

    def spectral(k1, xk):
        q = _dot(xk.astype(bf), gt_ref[k1])
        yr = q[:CP, :N2] - q[CP:, N2:]
        yi = q[:CP, N2:] + q[CP:, :N2]
        wr = w_scr[0, :, pl.ds(k1 * N2, N2)]
        wi = w_scr[1, :, pl.ds(k1 * N2, N2)]
        ypr = yr * wr - yi * wi
        ypi = yr * wi + yi * wr
        yp = jnp.concatenate([ypr, ypi], axis=0).astype(bf)
        r = _dot(yp, g_ref[k1])
        zr = r[:CP, :N2] + r[CP:, N2:]
        zi = r[CP:, :N2] - r[:CP, N2:]
        return jnp.concatenate([zr, zi], axis=0)

    for j in range(8):
        pa = p_scr[:, pl.ds(2 * j * N2, N2)]
        pb = p_scr[:, pl.ds((2 * j + 1) * N2, N2)]
        if j == 0:
            z_scr[:, pl.ds(0, N2)] = spectral(0, pa).astype(bf)
            z_scr[:, pl.ds(8 * N2, N2)] = spectral(8, pb).astype(bf)
        else:
            sw = jnp.concatenate([-pb[CP:], pb[:CP]], axis=0)
            za = spectral(j, pa + sw)
            zb = spectral(N1 - j, pa - sw)
            z_scr[:, pl.ds(j * N2, N2)] = (za + zb).astype(bf)
            z_scr[:, pl.ds((8 + j) * N2, N2)] = (za - zb).astype(bf)

    b_scr[:, pl.ds(0, 9 * N2)] = _dot(ci1_ref[...], z_scr[:, pl.ds(0, 9 * N2)])
    b_scr[:, pl.ds(9 * N2, 7 * N2)] = _dot(ci2_ref[...], z_scr[:, pl.ds(9 * N2, 7 * N2)])

    for rc in range(D // RB):
        rows = pl.ds(rc * RB, RB)
        pj = [b_scr[rows, pl.ds(j * N2, N2)] for j in range(9)]
        mj = [None] + [b_scr[rows, pl.ds((8 + j) * N2, N2)] for j in range(1, 8)]
        ys = _irdft16(pj, mj)
        for n in range(N1):
            cols = pl.ds(n * N2, N2)
            h_scr[rows, cols] = (x_ref[rows, cols].astype(f32)
                                 + ys[n].astype(bf).astype(f32)).astype(bf)

    hf = h_scr[...].astype(f32)
    mu2 = jnp.mean(hf, axis=0, keepdims=True)
    hc = hf - mu2
    rs2 = jax.lax.rsqrt(jnp.mean(hc * hc, axis=0, keepdims=True) + EPS)
    ln2_scr[...] = (hc * rs2).astype(bf)

    for cp in copies[7:]:
        cp.wait()
    for t in range(S // TS):
        cols = pl.ds(t * TS, TS)
        ln2 = ln2_scr[:, cols].T
        g = _dot(ln2, wg_ref[...]).astype(bf)
        u = _dot(ln2, wu_ref[...]).astype(bf)
        hh = (g.astype(f32) * u.astype(f32)).astype(bf)
        o = jax.lax.dot_general(wd_ref[...], hh, (((1,), (1,)), ((), ())),
                                preferred_element_type=f32)
        o_ref[:, cols] = (h_scr[:, cols].astype(f32)
                          + o.astype(bf).astype(f32)).astype(o_ref.dtype)


@jax.jit
def pallas_sequential_preLN__spectral_gfnet__glu_gated_bilinear__prompt_kernel(
    A_x: jax.Array,
    A_w_r: jax.Array,
    A_w_i: jax.Array,
    B_x: jax.Array,
    B_w_gate: jax.Array,
    B_w_up: jax.Array,
    B_w_down: jax.Array,
):
    del B_x
    xt = A_x.reshape(S, D).T
    consts = _constants()
    out = pl.pallas_call(
        _kernel,
        out_shape=jax.ShapeDtypeStruct((D, S), jnp.bfloat16),
        in_specs=[pl.BlockSpec(memory_space=pltpu.VMEM)] + [pl.BlockSpec(memory_space=pl.ANY)] * 10
                 + [pl.BlockSpec(memory_space=pltpu.VMEM)],
        scratch_shapes=[
            pltpu.VMEM((D, S), jnp.bfloat16),
            pltpu.VMEM((2 * CP, S), jnp.float32),
            pltpu.VMEM((2 * CP, S), jnp.bfloat16),
            pltpu.VMEM((D, S), jnp.float32),
            pltpu.VMEM((D, S), jnp.bfloat16),
            pltpu.VMEM((D, S), jnp.bfloat16),
            pltpu.VMEM((DF, S), jnp.bfloat16),
            pltpu.VMEM((DF, S), jnp.bfloat16),
            pltpu.VMEM((D, F), jnp.bfloat16),
            pltpu.VMEM((D, F), jnp.bfloat16),
            pltpu.VMEM((D, F), jnp.bfloat16),
            pltpu.VMEM((2 * CP, D), jnp.bfloat16),
            pltpu.VMEM((D, 2 * CP), jnp.bfloat16),
            pltpu.VMEM((D, 2 * CP), jnp.bfloat16),
            pltpu.VMEM((N1, N2, 2 * N2), jnp.bfloat16),
            pltpu.VMEM((N1, N2, 2 * N2), jnp.bfloat16),
            pltpu.VMEM((2, CP, S), jnp.float32),
            pltpu.SemaphoreType.DMA((10,)),
        ],
        compiler_params=pltpu.CompilerParams(vmem_limit_bytes=100 * 1024 * 1024),
    )(xt, A_w_r.T, A_w_i.T, B_w_gate, B_w_up, B_w_down.T, *consts)
    return out.T.reshape(1, S, D)
```
